```python
import os as _os
_os.environ.setdefault("JAX_PLATFORMS", "cpu")
import jax
import jax.numpy as jnp

def _softmax(x, axis=-1):
    return jax.nn.softmax(x, axis=axis)
def _gelu(x):
    return jax.nn.gelu(x, approximate=True)
def _silu(x):
    return jax.nn.silu(x)
def _sigmoid(x):
    return jax.nn.sigmoid(x)
def _layernorm(x, axis=-1, eps=1e-5):
    m = jnp.mean(x, axis=axis, keepdims=True)
    v = jnp.var(x, axis=axis, keepdims=True)
    return (x - m) / jnp.sqrt(v + eps)
def _scatter_add(tgt, idx, src, axis=0):
    return tgt.at[idx].add(src)
def _segment_sum(src, seg, n):
    return jax.ops.segment_sum(src, seg, n)
class _Rng:
    def __init__(self, key):
        self._k = key
    def _next(self):
        self._k, sub = jax.random.split(self._k)
        return sub
    def normal(self, shape):
        return jax.random.normal(self._next(), shape, dtype=jnp.bfloat16)
    def randint(self, lo, hi, shape):
        return jax.random.randint(self._next(), shape, lo, hi, dtype=jnp.int32)
    def uniform(self, shape, lo=0.0, hi=1.0):
        return jax.random.uniform(self._next(), shape, jnp.bfloat16, lo, hi)
    def permutation(self, n):
        return jax.random.permutation(self._next(), n)


kernel_name = 'concat_heads__sliding_local_dilated__compressed_kv_cla__prompt'

def setup_inputs():
    _rng = _Rng(jax.random.key(int.from_bytes(__import__("os").urandom(4), "little")))
    _w = (lambda a: (lambda t: t.astype(jnp.bfloat16) if jnp.issubdtype(t.dtype, jnp.floating) else t)(jnp.asarray(a)))
    def _A_setup():
        B, S, D = 1, 2048, 640
        return {
            "x": _w((lambda *s: _rng.normal(s) * 0.2)(B, S, D)),
            "wqkv": _w((lambda *s: _rng.normal(s) * 0.2)(D, 3 * D)),
            "wo": _w((lambda *s: _rng.normal(s) * 0.05)(D, D)),
        }
    _A_in = _A_setup()

    def _B_setup():
        B, H, Sq, Sk, D, M = 1, 32, 2048, 2048, 128, 640
        Dc = 4 * D
        return {
            "x": _w((lambda *s: _rng.normal(s) * 0.8)(B, Sq, M)),
            "c_kv": _w((lambda *s: _rng.normal(s) * 0.8)(B, Sk, Dc)),
            "w_q": _w((lambda *s: _rng.normal(s) * 1.6)(M, H, D) * (M ** -0.5)),
            "w_uk": _w((lambda *s: _rng.normal(s) * 1.6)(Dc, H, D) * (Dc ** -0.5)),
            "w_uv": _w((lambda *s: _rng.normal(s) * 0.8)(Dc, H, D) * (Dc ** -0.5)),
            "w_o": _w((lambda *s: _rng.normal(s) * 0.8)(H, D, M) * ((H * D) ** -0.5)),
        }
    _B_in = _B_setup()

    return {
        "A_x": _A_in["x"],
        "A_wqkv": _A_in["wqkv"],
        "A_wo": _A_in["wo"],
        "B_x": _B_in["x"],
        "B_c_kv": _B_in["c_kv"],
        "B_w_q": _B_in["w_q"],
        "B_w_uk": _B_in["w_uk"],
        "B_w_uv": _B_in["w_uv"],
        "B_w_o": _B_in["w_o"],
    }

def reference(A_x, A_wqkv, A_wo, B_x, B_c_kv, B_w_q, B_w_uk, B_w_uv, B_w_o):
    def _A_ref(x, wqkv, wo):
        B, S, D = x.shape
        H = 32; Dh = D // H
        W, dil = 8, 2
        qkv = (lambda x, *d: x.transpose(*d))((x @ wqkv).reshape(B, S, 3, H, Dh), 2, 0, 3, 1, 4)
        q, k, v = qkv[0], qkv[1], qkv[2]
        scale = Dh ** -0.5
        pos = jnp.arange(S)
        off = jnp.arange(W) * dil
        idx = pos[:, None] - off[None, :]
        mask = idx >= 0
        idx_c = jnp.where(mask, idx, 0).reshape(-1)
        kg = k[:, :, idx_c, :].reshape(B, H, S, W, Dh)
        vg = v[:, :, idx_c, :].reshape(B, H, S, W, Dh)
        logits = jnp.einsum("bhsd,bhswd->bhsw", q, kg) * scale
        logits = jnp.where(mask[None, None, :, :], logits, -1e9)
        attn = _softmax(logits, axis=-1)
        o = jnp.einsum("bhsw,bhswd->bhsd", attn, vg)
        return (lambda x, *d: x.transpose(*d))(o, 0, 2, 1, 3).reshape(B, S, D) @ wo

    def _B_ref(x, c_kv, w_q, w_uk, w_uv, w_o):
        B, Sq, M = x.shape[0], x.shape[1], x.shape[2]
        Sk = c_kv.shape[1]
        H, D = w_q.shape[1], w_q.shape[2]
        q = jnp.einsum("bqm,mhd->bhqd", x, w_q)
        k = jnp.einsum("bkc,chd->bhkd", c_kv, w_uk)
        v = jnp.einsum("bkc,chd->bhkd", c_kv, w_uv)
        scores = jnp.einsum("bhqd,bhkd->bhqk", q, k) * (D ** -0.5)
        off = Sk - Sq
        qi = jnp.arange(Sq)[:, None]
        kj = jnp.arange(Sk)[None, :]
        cmask = kj <= (qi + off)
        scores = jnp.where(cmask[None, None], scores, -1e9)
        p = _softmax(scores, axis=-1)
        ctx = jnp.einsum("bhqk,bhkd->bhqd", p, v)
        return jnp.einsum("bhqd,hdm->bqm", ctx, w_o)

    a = _A_ref(A_x, A_wqkv, A_wo)
    b = _B_ref(B_x, B_c_kv, B_w_q, B_w_uk, B_w_uv, B_w_o)
    return jnp.concatenate([a, b], axis=-1)
```

```python
import jax
import jax.numpy as jnp
import numpy as np
import jax.experimental.pallas as pl
import jax.experimental.pallas.tpu as pltpu

S = 2048
DM = 640
HA, DHA = 32, 20
WIN, DIL = 8, 2
PAD = 16
HB, DB, DC = 32, 128, 512
NP = HB // 2
RA = 256
TQ = 256
RP = 512
RO = 256
LOG2E = 1.4426950408889634
F32, BF16 = jnp.float32, jnp.bfloat16
NT = (((1,), (1,)), ((), ()))


def _dot(a, b):
    return jnp.dot(a, b, preferred_element_type=F32)


def _iota(shape, d):
    return jax.lax.broadcasted_iota(jnp.int32, shape, d)


def _pair_weights(w_ref, i):
    w = w_ref.bitcast(jnp.uint32)[:, i, :]
    lo = pltpu.bitcast(w << 16, F32).astype(BF16)
    hi = pltpu.bitcast(w & jnp.uint32(0xFFFF0000), F32).astype(BF16)
    return jnp.concatenate([lo, hi], axis=1)


def _branch_a(ax, wqkv, wo, ks, vs, seg, segt, oa):
    nt = DM // 128
    r, c = _iota((DM, 128), 0), _iota((DM, 128), 1)
    rt, ct = _iota((128, DM), 1), _iota((128, DM), 0)
    for w in range(4):
        h = c - w * HA
        seg[w] = ((r >= h * DHA) & (r < (h + 1) * DHA) & (h >= 0) & (h < HA)).astype(F32).astype(BF16)
        h = ct - w * HA
        segt[w] = ((rt >= h * DHA) & (rt < (h + 1) * DHA) & (h >= 0) & (h < HA)).astype(F32).astype(BF16)

    def kv_body(ci, _):
        r0 = pl.multiple_of(ci * RP, RP)
        kv = _dot(ax[pl.ds(r0, RP), :], wqkv[:, DM:])
        for j in range(nt):
            ks[j, pl.ds(PAD + r0, RP), :] = kv[:, j * 128:(j + 1) * 128]
            vs[j, pl.ds(PAD + r0, RP), :] = kv[:, DM + j * 128:DM + (j + 1) * 128]
        return 0

    jax.lax.fori_loop(0, S // RP, kv_body, 0)
    for j in range(nt):
        ks[j, 0:PAD, :] = jnp.broadcast_to(ks[j, PAD:PAD + 1, :], (PAD, 128))
        vs[j, 0:PAD, :] = jnp.broadcast_to(vs[j, PAD:PAD + 1, :], (PAD, 128))

    def body(ci, _):
        r0 = pl.multiple_of(ci * RA, RA)
        q = _dot(ax[pl.ds(r0, RA), :], wqkv[:, :DM]) * (DHA ** -0.5 * LOG2E)
        pos = r0 + _iota((RA, 128), 0)
        tap = _iota((RA, 128), 1) // HA
        halves = []
        for g in range(2):
            acc = None
            for w in range(4):
                off = PAD - DIL * (4 * g + w)
                kk = jnp.concatenate([ks[j, pl.ds(r0 + off, RA), :] for j in range(nt)], axis=1)
                d = _dot((q * kk).astype(BF16), seg[w])
                acc = d if acc is None else acc + d
            halves.append(jnp.where(pos - DIL * (tap + 4 * g) >= 0, acc, -1e9 * LOG2E))
        m = jnp.maximum(halves[0], halves[1])
        m = jnp.maximum(m, pltpu.roll(m, 64, 1))
        m = jnp.maximum(m, pltpu.roll(m, 32, 1))
        e = [jnp.exp2(x - m) for x in halves]
        l = e[0] + e[1]
        l = l + pltpu.roll(l, 64, 1)
        l = l + pltpu.roll(l, 32, 1)
        inv = 1.0 / l
        o = None
        for g in range(2):
            p = (e[g] * inv).astype(BF16)
            for w in range(4):
                off = PAD - DIL * (4 * g + w)
                vv = jnp.concatenate([vs[j, pl.ds(r0 + off, RA), :] for j in range(nt)], axis=1)
                t = _dot(p, segt[w]) * vv
                o = t if o is None else o + t
        oa[pl.ds(r0, RA), :] = _dot(o.astype(BF16), wo[...]).astype(BF16)
        return 0

    jax.lax.fori_loop(0, S // RA, body, 0)


def _branch_b_pair(i, bx, ckv, wq, wuk, wuv, qs, kss, vss, ctx):
    wq2, wk2, wv2 = _pair_weights(wq, i), _pair_weights(wuk, i), _pair_weights(wuv, i)
    for c in range(S // RP):
        rows = slice(c * RP, (c + 1) * RP)
        qs[rows, :] = (_dot(bx[rows, :], wq2) * (DB ** -0.5 * LOG2E)).astype(BF16)
        kss[rows, :] = _dot(ckv[rows, :], wk2).astype(BF16)
        vss[rows, :] = _dot(ckv[rows, :], wv2).astype(BF16)
    causal = _iota((TQ, TQ), 1) <= _iota((TQ, TQ), 0)
    for qi in range(S // TQ):
        rows = slice(qi * TQ, (qi + 1) * TQ)
        n0 = qi * TQ
        for hh in range(2):
            cols = slice(hh * DB, (hh + 1) * DB)
            q = qs[rows, cols]
            sd = jax.lax.dot_general(q, kss[rows, cols], NT, preferred_element_type=F32)
            sd = jnp.where(causal, sd, -1e9 * LOG2E)
            m = jnp.max(sd, axis=1, keepdims=True)
            if qi:
                sf = jax.lax.dot_general(q, kss[0:n0, cols], NT, preferred_element_type=F32)
                m = jnp.maximum(m, jnp.max(sf, axis=1, keepdims=True))
            pd = jnp.exp2(sd - m)
            l = jnp.sum(pd, axis=1, keepdims=True)
            acc = _dot(pd.astype(BF16), vss[rows, cols])
            if qi:
                pf = jnp.exp2(sf - m)
                l = l + jnp.sum(pf, axis=1, keepdims=True)
                acc = acc + _dot(pf.astype(BF16), vss[0:n0, cols])
            ctx[i, rows, cols] = (acc * (1.0 / l)).astype(BF16)


def _kernel(ax_h, wqkv_h, awo_h, bx_h, ckv_h, wq_h, wuk_h, wuv_h, bwo_h, out_h,
            ax, wqkv, awo, bx, ckv, wq, wuk, wuv, bwo,
            ks, vs, seg, segt, oa, ob, qs, kss, vss, ctx, isem, osem):
    srcs = (ax_h, wqkv_h, awo_h, bx_h, ckv_h, wq_h, wuk_h, wuv_h, bwo_h)
    dsts = (ax, wqkv, awo, bx, ckv, wq, wuk, wuv, bwo)
    cps = [pltpu.make_async_copy(s, d, isem.at[n]) for n, (s, d) in enumerate(zip(srcs, dsts))]
    for cp in cps:
        cp.start()
    for cp in cps[:3]:
        cp.wait()
    _branch_a(ax, wqkv, awo, ks, vs, seg, segt, oa)
    a_out = pltpu.make_async_copy(oa, out_h.at[:, 0:DM], osem.at[0])
    a_out.start()
    for cp in cps[3:8]:
        cp.wait()

    def pair_body(i, _):
        _branch_b_pair(i, bx, ckv, wq, wuk, wuv, qs, kss, vss, ctx)
        return 0

    jax.lax.fori_loop(0, NP, pair_body, 0)
    cps[8].wait()
    outs = []
    for c in range(S // RO):
        rows = slice(c * RO, (c + 1) * RO)
        acc = None
        for i in range(NP):
            d = _dot(ctx[i, rows, :], bwo[i * 2 * DB:(i + 1) * 2 * DB, :])
            acc = d if acc is None else acc + d
        ob[rows, :] = acc.astype(BF16)
        cp = pltpu.make_async_copy(ob.at[rows, :], out_h.at[rows, DM:2 * DM], osem.at[1 + c])
        cp.start()
        outs.append(cp)
    a_out.wait()
    for cp in outs:
        cp.wait()


@jax.jit
def pallas_concat_heads__sliding_local_dilated__compressed_kv_cla__prompt_kernel(
    A_x: jax.Array,
    A_wqkv: jax.Array,
    A_wo: jax.Array,
    B_x: jax.Array,
    B_c_kv: jax.Array,
    B_w_q: jax.Array,
    B_w_uk: jax.Array,
    B_w_uv: jax.Array,
    B_w_o: jax.Array,
):
    args = (A_x.reshape(S, DM), A_wqkv, A_wo, B_x.reshape(S, DM), B_c_kv.reshape(S, DC),
            B_w_q, B_w_uk, B_w_uv, B_w_o.reshape(HB * DB, DM))
    vm = pltpu.VMEM
    scratch = [vm(a.shape, BF16) for a in args] + [
        vm((DM // 128, PAD + S, 128), F32), vm((DM // 128, PAD + S, 128), F32),
        vm((4, DM, 128), BF16), vm((4, 128, DM), BF16),
        vm((S, DM), BF16), vm((S, DM), BF16),
        vm((S, 2 * DB), BF16), vm((S, 2 * DB), BF16), vm((S, 2 * DB), BF16),
        vm((NP, S, 2 * DB), BF16),
        pltpu.SemaphoreType.DMA((9,)), pltpu.SemaphoreType.DMA((1 + S // RO,)),
    ]
    out = pl.pallas_call(
        _kernel,
        out_shape=jax.ShapeDtypeStruct((S, 2 * DM), BF16),
        in_specs=[pl.BlockSpec(memory_space=pl.ANY)] * 9,
        out_specs=pl.BlockSpec(memory_space=pl.ANY),
        scratch_shapes=scratch,
        compiler_params=pltpu.CompilerParams(vmem_limit_bytes=110 * 1024 * 1024),
    )(*args)
    return out.reshape(1, S, 2 * DM)
```

```python
import jax
import jax.numpy as jnp
import jax.experimental.pallas as pl
import jax.experimental.pallas.tpu as pltpu

S = 2048
DM = 640
HA, DHA = 32, 20
WIN, DIL = 8, 2
PAD = 16
HB, DB, DC = 32, 128, 512
NP = HB // 2
RA = 512
GA = 32
TQ = 256
RO = 256
DIST = 5
LOG2E = 1.4426950408889634
NEG = -1e9 * LOG2E
F32, BF16 = jnp.float32, jnp.bfloat16
NT = (((1,), (1,)), ((), ()))


def _dot(a, b):
    return jnp.dot(a, b, preferred_element_type=F32)


def _iota(shape, d):
    return jax.lax.broadcasted_iota(jnp.int32, shape, d)


def _pair_weights(w_ref, i):
    w = w_ref[i // 8, pl.ds(i % 8, w_ref.shape[1] // 8, stride=8), :]
    lo = pltpu.bitcast(w << 16, F32).astype(BF16)
    hi = pltpu.bitcast(w & jnp.uint32(0xFFFF0000), F32).astype(BF16)
    return jnp.concatenate([lo, hi], axis=1)


def _recip(l):
    r = pl.reciprocal(l, approx=True)
    return r * (2.0 - l * r)


def _nt(a, b):
    return jax.lax.dot_general(a, b, NT, preferred_element_type=F32)


def _branch_a(ax, wqkv, wo, wt, wtp, wop, qa, ks, vs, oc, oa, wait, filler):
    nt = DM // 128

    def prep(p):
        for j in range(nt):
            if p < 3:
                t = wqkv[:, p * DM + j * 128:p * DM + (j + 1) * 128].astype(F32).T
                for jj in range(nt):
                    wt[jj, p * DM + j * 128:p * DM + (j + 1) * 128, :] = t[:, jj * 128:(jj + 1) * 128]
            else:
                wt[j, p * DM:(p + 1) * DM, :] = wo[:, j * 128:(j + 1) * 128].astype(F32)
        dst, base = (wtp, p * DM) if p < 3 else (wop, 0)
        for d in range(DHA):
            for j in range(nt):
                t = wt[j, pl.ds(p * DM + d, HA, stride=DHA), :]
                dst[base + d * HA:base + (d + 1) * HA, j * 128:(j + 1) * 128] = t.astype(BF16)

    def project(c, p, dep=None):
        y = _nt(tie(ax[c * RA:(c + 1) * RA, :], dep), wtp[p * DM:(p + 1) * DM, :])
        for j in range(nt):
            t = y[:, j * 128:(j + 1) * 128]
            if p == 0:
                qa[j, c * RA:(c + 1) * RA, :] = t * (DHA ** -0.5 * LOG2E)
                continue
            dst = ks if p == 1 else vs
            dst[j, PAD + c * RA:PAD + (c + 1) * RA, :] = t
            if c == 0:
                dst[j, 0:PAD, :] = jnp.broadcast_to(t[0:1, :], (PAD, 128))

    def tie(x, r_end):
        if r_end is None:
            return x
        top = jnp.where(never, oc[r_end - 16:r_end, 0:128], x[:16, :128])
        return jnp.concatenate([jnp.concatenate([top, x[:16, 128:]], axis=1), x[16:]], axis=0)

    def attend(r0):
        q = [qa[j, r0:r0 + GA, :] for j in range(nt)]
        half = WIN // 2

        def taps(ref, j, w):
            o = r0 + PAD - DIL * (w + half)
            t = ref[j, o:o + GA + 8, :]
            return t[8:], t[:GA]

        lg = [None] * WIN
        for w in range(half):
            for j in range(nt):
                for u, t in zip((w, w + half), taps(ks, j, w)):
                    lg[u] = q[j] * t if j == 0 else lg[u] + q[j] * t
        for w in range(WIN):
            x = lg[w] + pltpu.roll(lg[w], 64, 1)
            x = x + pltpu.roll(x, 32, 1)
            if r0 < DIL * w:
                x = jnp.where(_iota((GA, 128), 0) + r0 >= DIL * w, x, NEG)
            lg[w] = x
        m = lg[0]
        for x in lg[1:]:
            m = jnp.maximum(m, x)
        e = [jnp.exp2(x - m) for x in lg]
        l = e[0]
        for x in e[1:]:
            l = l + x
        inv = _recip(l)
        for j in range(nt):
            acc = None
            for w in range(half):
                t0, t1 = taps(vs, j, w)
                t = e[w] * t0 + e[w + half] * t1
                acc = t if acc is None else acc + t
            oc[r0:r0 + GA, j * 128:(j + 1) * 128] = (acc * inv).astype(BF16)

    wait(0)
    prep(1)
    wait(1)
    project(0, 1)
    prep(2)
    wait(2)
    project(0, 2)
    prep(0)
    prep(3)
    project(0, 0)
    wait(3)
    nc = S // RA
    never = _iota((16, 128), 0) < 0

    def dep(c, p):
        r = c * RA + (p - 1) * (RA // 4)
        return r if r > 0 else None

    def out_a(c, r_end):
        rows = slice(c * RA, (c + 1) * RA)
        oa[rows, :] = _dot(tie(oc[rows, :], r_end), wop[...]).astype(BF16)

    for c in range(nc):
        for p in range(4):
            if c + 1 < nc and p < 3:
                project(c + 1, p, dep(c, p))
            elif c + 1 == nc and p == 0:
                filler()
            elif c and p == 3:
                out_a(c - 1, dep(c, p))
            for r0 in range(c * RA + p * RA // 4, c * RA + (p + 1) * RA // 4, GA):
                attend(r0)
    out_a(nc - 1, None)


def _stage_weights(i, wq, wuk, wuv, w2):
    w2[0:DM, :] = _pair_weights(wq, i)
    w2[DM:DM + DC, :] = _pair_weights(wuk, i)
    w2[DM + DC:, :] = _pair_weights(wuv, i)


def _branch_b_pair(i, bx, ckv, wq, wuk, wuv, w2, qs, kss, vss, ctx, mode):
    def proj(c, parts=(0, 1, 2)):
        rows = slice(c * TQ, (c + 1) * TQ)
        if 0 in parts:
            qs[rows, :] = (_dot(bx[rows, :], w2[0:DM, :]) * (DB ** -0.5 * LOG2E)).astype(BF16)
        if 1 in parts:
            kss[:, rows] = _dot(ckv[rows, :], w2[DM:DM + DC, :]).T.astype(BF16)
        if 2 in parts:
            vss[rows, :] = _dot(ckv[rows, :], w2[DM + DC:, :]).astype(BF16)

    ng = TQ // 128
    causal = _iota((128, 128), 1) <= _iota((128, 128), 0)
    blocks = [(qi, hh) for qi in reversed(range(S // TQ)) for hh in range(2)]
    never = _iota((16, DB), 0) < 0

    def load_q(r):
        qi, hh = blocks[r]
        q = qs[qi * TQ:(qi + 1) * TQ, hh * DB:(hh + 1) * DB]
        if r < DIST:
            return q
        pi, ph = blocks[r - DIST]
        done = ctx[i, pi * TQ + TQ - 16:(pi + 1) * TQ, ph * DB:(ph + 1) * DB]
        return jnp.concatenate([jnp.where(never, done, q[:16]), q[16:]], axis=0)

    def lower(op, x, y):
        n = x.shape[0] - y.shape[0]
        return jnp.concatenate([x[:n], op(x[n:], y)], axis=0) if n else op(x, y)

    def scores(r, q):
        qi, hh = blocks[r]
        n0, cols = qi * TQ, slice(hh * DB, (hh + 1) * DB)
        sf = _dot(q, kss[cols, 0:n0]) if qi else None
        sd, mx = [], None
        for t in range(ng):
            x = _dot(q[t * 128:], kss[cols, n0 + t * 128:n0 + (t + 1) * 128])
            top = jnp.where(causal, x[:128], NEG)
            x = jnp.concatenate([top, x[128:]], axis=0) if t + 1 < ng else top
            sd.append(x)
            mx = lower(jnp.maximum, mx, x) if t else x
        for t in range(n0 // 128):
            mx = jnp.maximum(mx, sf[:, t * 128:(t + 1) * 128])
        return sd, sf, jnp.max(mx, axis=1, keepdims=True)

    def finish(r, sd, sf, m):
        qi, hh = blocks[r]
        n0, cols = qi * TQ, slice(hh * DB, (hh + 1) * DB)
        acc = ls = None
        if qi:
            pf = jnp.exp2(sf - m)
            for t in range(n0 // 128):
                ls = ls + pf[:, t * 128:(t + 1) * 128] if t else pf[:, 0:128]
            acc = _dot(pf.astype(BF16), vss[0:n0, cols])
        for t in range(ng):
            p = jnp.exp2(sd[t] - m[t * 128:])
            d = _dot(p.astype(BF16), vss[n0 + t * 128:n0 + (t + 1) * 128, cols])
            ls = p if ls is None else lower(jnp.add, ls, p)
            acc = d if acc is None else lower(jnp.add, acc, d)
        inv = _recip(jnp.sum(ls, axis=1, keepdims=True))
        ctx[i, n0:n0 + TQ, cols] = (acc * inv).astype(BF16)

    nb = len(blocks)
    if mode == "proj":
        for c in range(S // TQ):
            proj(c)
        return
    nxt = mode == "both"
    if nxt:
        _stage_weights(i + 1, wq, wuk, wuv, w2)
    sc = [scores(0, load_q(0))]
    todo = [(c, parts) for c in reversed(range(S // TQ)) for parts in ((1, 2), (0,))]
    for r in range(nb):
        left = [qi for qi, _ in blocks[r:]]
        ready = [t for t in todo if (t[0] not in left if t[1] == (0,) else t[0] > max(left))]
        if r + 1 < nb:
            sc.append(scores(r + 1, load_q(r + 1)))
        for t in (ready[:1] if nxt else ()):
            proj(*t)
            todo.remove(t)
        finish(r, *sc[r])
    for t in (todo if nxt else ()):
        proj(*t)


def _kernel(ax_h, wqkv_h, awo_h, bx_h, ckv_h, wq_h, wuk_h, wuv_h, bwo_h, out_h,
            ax, wqkv, awo, bx, ckv, wq, wuk, wuv, bwo,
            wt, wtp, wop, qa, ks, vs, oc, oa, ob, w2, qs, kss, vss, ctx, isem, osem):
    def copy(src, dst, n):
        return pltpu.make_async_copy(src, dst, isem.at[n])

    def head_weights(g):
        return [copy(s.bitcast(jnp.uint32).at[:, 8 * g:8 * g + 8, :], d.at[g].reshape(s.shape[0], 8, DB), 9 + 3 * g + n)
                for n, (s, d) in enumerate(((wq_h, wq), (wuk_h, wuk), (wuv_h, wuv)))]

    b_in = [copy(bx_h, bx, 3), copy(ckv_h, ckv, 4)] + head_weights(0)
    b_late, wo_cp = head_weights(1), copy(bwo_h, bwo, 8)
    wcp = [pltpu.make_async_copy(wqkv_h.at[:, p * DM:(p + 1) * DM], wqkv.at[:, p * DM:(p + 1) * DM], isem.at[5 + p])
           for p in range(3)]
    x0 = pltpu.make_async_copy(ax_h.at[:RA], ax.at[:RA], isem.at[1])
    x1 = pltpu.make_async_copy(ax_h.at[RA:], ax.at[RA:], isem.at[0])
    stages = ([wcp[1]], [x0, wcp[2]], [wcp[0], copy(awo_h, awo, 2)], [x1], b_in)

    def start(cps):
        for cp in cps:
            cp.start()

    def finish(cps):
        for cp in cps:
            cp.wait()

    start(stages[0])

    def wait(n):
        if n < 3:
            start(stages[n + 1])
        finish(stages[n])
        if n == 3:
            start(stages[n + 1])

    def filler():
        finish(b_in)
        start(b_late)
        _stage_weights(0, wq, wuk, wuv, w2)
        _branch_b_pair(0, bx, ckv, wq, wuk, wuv, w2, qs, kss, vss, ctx, "proj")

    _branch_a(ax, wqkv, awo, wt, wtp, wop, qa, ks, vs, oc, oa, wait, filler)
    a_out = pltpu.make_async_copy(oa, out_h.at[:, 0:DM], osem.at[0])
    a_out.start()
    finish(b_late)
    wo_cp.start()

    def pair_body(i, _):
        _branch_b_pair(i, bx, ckv, wq, wuk, wuv, w2, qs, kss, vss, ctx, "both")
        return 0

    jax.lax.fori_loop(0, NP - 1, pair_body, 0)
    _branch_b_pair(NP - 1, bx, ckv, wq, wuk, wuv, w2, qs, kss, vss, ctx, "attn")
    wo_cp.wait()
    outs = [a_out]
    for c in range(S // RO):
        rows = slice(c * RO, (c + 1) * RO)
        acc = None
        for i in range(NP):
            d = _dot(ctx[i, rows, :], bwo[i * 2 * DB:(i + 1) * 2 * DB, :])
            acc = d if acc is None else acc + d
        ob[rows, :] = acc.astype(BF16)
        outs.append(pltpu.make_async_copy(ob.at[rows, :], out_h.at[rows, DM:2 * DM], osem.at[1 + c]))
        outs[-1].start()
    finish(outs)


@jax.jit
def pallas_concat_heads__sliding_local_dilated__compressed_kv_cla__prompt_kernel(
    A_x: jax.Array,
    A_wqkv: jax.Array,
    A_wo: jax.Array,
    B_x: jax.Array,
    B_c_kv: jax.Array,
    B_w_q: jax.Array,
    B_w_uk: jax.Array,
    B_w_uv: jax.Array,
    B_w_o: jax.Array,
):
    args = (A_x.reshape(S, DM), A_wqkv, A_wo, B_x.reshape(S, DM), B_c_kv.reshape(S, DC),
            B_w_q, B_w_uk, B_w_uv, B_w_o.reshape(HB * DB, DM))
    vm = pltpu.VMEM
    scratch = [vm(a.shape, BF16) if a.ndim == 2 else vm((NP // 8, a.shape[0] * 8, DB), jnp.uint32) for a in args] + [
        vm((DM // 128, 4 * DM, 128), F32), vm((3 * DM, DM), BF16), vm((DM, DM), BF16),
        vm((DM // 128, S, 128), F32), vm((DM // 128, PAD + S, 128), F32), vm((DM // 128, PAD + S, 128), F32),
        vm((S, DM), BF16),
        vm((S, DM), BF16), vm((S, DM), BF16), vm((DM + 2 * DC, 2 * DB), BF16),
        vm((S, 2 * DB), BF16), vm((2 * DB, S), BF16), vm((S, 2 * DB), BF16),
        vm((NP, S, 2 * DB), BF16),
        pltpu.SemaphoreType.DMA((15,)), pltpu.SemaphoreType.DMA((1 + S // RO,)),
    ]
    out = pl.pallas_call(
        _kernel,
        out_shape=jax.ShapeDtypeStruct((S, 2 * DM), BF16),
        in_specs=[pl.BlockSpec(memory_space=pl.ANY)] * 9,
        out_specs=pl.BlockSpec(memory_space=pl.ANY),
        scratch_shapes=scratch,
        compiler_params=pltpu.CompilerParams(vmem_limit_bytes=110 * 1024 * 1024),
    )(*args)
    return out.reshape(1, S, 2 * DM)
```
